```python
import os as _os
_os.environ.setdefault("JAX_PLATFORMS", "cpu")
import jax
import jax.numpy as jnp

def _softmax(x, axis=-1):
    return jax.nn.softmax(x, axis=axis)
def _gelu(x):
    return jax.nn.gelu(x, approximate=True)
def _silu(x):
    return jax.nn.silu(x)
def _sigmoid(x):
    return jax.nn.sigmoid(x)
def _layernorm(x, axis=-1, eps=1e-5):
    m = jnp.mean(x, axis=axis, keepdims=True)
    v = jnp.var(x, axis=axis, keepdims=True)
    return (x - m) / jnp.sqrt(v + eps)
def _scatter_add(tgt, idx, src, axis=0):
    return tgt.at[idx].add(src)
def _segment_sum(src, seg, n):
    return jax.ops.segment_sum(src, seg, n)
class _Rng:
    def __init__(self, key):
        self._k = key
    def _next(self):
        self._k, sub = jax.random.split(self._k)
        return sub
    def normal(self, shape):
        return jax.random.normal(self._next(), shape, dtype=jnp.bfloat16)
    def randint(self, lo, hi, shape):
        return jax.random.randint(self._next(), shape, lo, hi, dtype=jnp.int32)
    def uniform(self, shape, lo=0.0, hi=1.0):
        return jax.random.uniform(self._next(), shape, jnp.bfloat16, lo, hi)
    def permutation(self, n):
        return jax.random.permutation(self._next(), n)


kernel_name = 'concat_heads__gqa_block_cached__mha_block_cached__near_ridge'

def setup_inputs():
    _rng = _Rng(jax.random.key(int.from_bytes(__import__("os").urandom(4), "little")))
    _w = (lambda a: (lambda t: t.astype(jnp.bfloat16) if jnp.issubdtype(t.dtype, jnp.floating) else t)(jnp.asarray(a)))
    def _A_setup():
        B, Sq, D = 16, 32, 1024
        Hq, Hkv, Sk, Dh = 32, 4, 32, 128
        assert Hq % Hkv == 0, (Hq, Hkv)
        return {
            "x": _w((lambda *s: _rng.normal(s) * 0.8)(B, Sq, D)),
            "k_cache": _w((lambda *s: _rng.normal(s) * 0.8)(B, Hkv, Sk, Dh)),
            "v_cache": _w((lambda *s: _rng.normal(s) * 0.05)(B, Hkv, Sk, Dh)),
            "wq": _w((lambda *s: _rng.normal(s) * 0.8)(D, Hq * Dh) * (D ** -0.5)),
            "wo": _w((lambda *s: _rng.normal(s) * 0.05)(Hq * Dh, D) * ((Hq * Dh) ** -0.5)),
        }
    _A_in = _A_setup()

    def _B_setup():
        B, Sq, D = 16, 32, 1024
        H, Sk, Dh = 32, 32, 128
        return {
            "x": _w((lambda *s: _rng.normal(s) * 0.8)(B, Sq, D)),
            "k_cache": _w((lambda *s: _rng.normal(s) * 0.8)(B, H, Sk, Dh)),
            "v_cache": _w((lambda *s: _rng.normal(s) * 0.05)(B, H, Sk, Dh)),
            "wq": _w((lambda *s: _rng.normal(s) * 0.8)(D, H * Dh) * (D ** -0.5)),
            "wo": _w((lambda *s: _rng.normal(s) * 0.05)(H * Dh, D) * ((H * Dh) ** -0.5)),
        }
    _B_in = _B_setup()

    return {
        "A_x": _A_in["x"],
        "A_k_cache": _A_in["k_cache"],
        "A_v_cache": _A_in["v_cache"],
        "A_wq": _A_in["wq"],
        "A_wo": _A_in["wo"],
        "B_x": _B_in["x"],
        "B_k_cache": _B_in["k_cache"],
        "B_v_cache": _B_in["v_cache"],
        "B_wq": _B_in["wq"],
        "B_wo": _B_in["wo"],
    }

def reference(A_x, A_k_cache, A_v_cache, A_wq, A_wo, B_x, B_k_cache, B_v_cache, B_wq, B_wo):
    def _A_ref(x, k_cache, v_cache, wq, wo):
        B, Sq, D = x.shape
        Hq, Dh = 32, 128
        Hkv = k_cache.shape[1]
        rep = Hq // Hkv
        q = (lambda x, *d: x.transpose(*d))((x @ wq).reshape(B, Sq, Hq, Dh), 0, 2, 1, 3)
        k = jnp.repeat(k_cache, rep, axis=1)
        v = jnp.repeat(v_cache, rep, axis=1)
        scores = jnp.einsum("bhqd,bhkd->bhqk", q, k) * (Dh ** -0.5)
        p = _softmax(scores, axis=-1)
        o = jnp.einsum("bhqk,bhkd->bhqd", p, v)
        return (lambda x, *d: x.transpose(*d))(o, 0, 2, 1, 3).reshape(B, Sq, Hq * Dh) @ wo

    def _B_ref(x, k_cache, v_cache, wq, wo):
        B, Sq, D = x.shape
        H, Dh = 32, 128
        q = (lambda x, *d: x.transpose(*d))((x @ wq).reshape(B, Sq, H, Dh), 0, 2, 1, 3)
        scores = jnp.einsum("bhqd,bhkd->bhqk", q, k_cache) * (Dh ** -0.5)
        p = _softmax(scores, axis=-1)
        o = jnp.einsum("bhqk,bhkd->bhqd", p, v_cache)
        return (lambda x, *d: x.transpose(*d))(o, 0, 2, 1, 3).reshape(B, Sq, H * Dh) @ wo

    a = _A_ref(A_x, A_k_cache, A_v_cache, A_wq, A_wo)
    b = _B_ref(B_x, B_k_cache, B_v_cache, B_wq, B_wo)
    return jnp.concatenate([a, b], axis=-1)
```

```python
import functools
import jax
import jax.numpy as jnp
from jax import lax
import jax.experimental.pallas as pl
import jax.experimental.pallas.tpu as pltpu

B, SQ, D = 16, 32, 1024
H, SK, DH = 32, 32, 128
M = B * SQ
G = 4
NG = H // G
BF = jnp.bfloat16
F32 = jnp.float32
NT = (((1,), (1,)), ((), ()))


def _kernel(ax, ak, av, awq, awo, bx, bk, bv, bwq, bwo, out,
            x_v, wq_v, wo_v, ak_v, av_v, bk_v, bv_v, acc, o_v, sems, osems, *, ahead):
    stages = [(br, g) for br in range(2) for g in range(NG)]
    copies = {}
    order = []

    def add(name, src, dst):
        copies[name] = pltpu.make_async_copy(src, dst, sems.at[len(copies)])

    for br, (x, wq, wo) in enumerate(((ax, awq, awo), (bx, bwq, bwo))):
        add(("x", br), x, x_v.at[br])
        for g in range(NG):
            add(("wq", br, g), wq.at[:, pl.ds(g * G * DH, G * DH)], wq_v.at[br, g])
            add(("wo", br, g), wo.at[pl.ds(g * G * DH, G * DH), :], wo_v.at[br, g])
    add(("k", 0), ak, ak_v)
    add(("v", 0), av, av_v)
    for g in range(NG):
        rows = pl.ds(g * G * SK, G * SK)
        add(("k", 1, g), bk.at[:, rows, :], bk_v.at[g])
        add(("v", 1, g), bv.at[:, rows, :], bv_v.at[g])

    def needs(t):
        r = []
        if t < len(stages):
            br, g = stages[t]
            if g == 0:
                r.append(("x", br))
            r.append(("wq", br, g))
            if br == 0 and g == 0:
                r.append(("k", 0))
            if br == 1:
                r.append(("k", 1, g))
        if t >= 1:
            br, g = stages[t - 1]
            if br == 0 and g == 0:
                r.append(("v", 0))
            if br == 1:
                r.append(("v", 1, g))
            r.append(("wo", br, g))
        return r

    lane_blk = lax.broadcasted_iota(jnp.int32, (SK, 128), 1) // 32
    scale = DH ** -0.5

    def qproj(br, g):
        return jnp.dot(x_v[br], wq_v[br, g], preferred_element_type=F32).astype(BF)

    def scores(br, g, q):
        ps = []
        for bb in range(B // 4):
            pts = []
            for b in range(4 * bb, 4 * bb + 4):
                qs = jnp.concatenate(
                    [q[b * SQ:(b + 1) * SQ, j * DH:(j + 1) * DH] for j in range(G)], axis=0)
                if br == 0:
                    kv = (g * G) // 8
                    st = lax.dot_general(ak_v[b, kv * SK:(kv + 1) * SK, :], qs, NT,
                                         preferred_element_type=F32)
                else:
                    full = lax.dot_general(bk_v[g, b], qs, NT, preferred_element_type=F32)
                    st = full[0:SK]
                    for j in range(1, G):
                        st = jnp.where(lane_blk == j, full[j * SK:(j + 1) * SK], st)
                m = jnp.max(st, axis=0, keepdims=True)
                e = jnp.exp((st - m) * scale)
                s = jnp.sum(e, axis=0, keepdims=True)
                pts.append(e * (1.0 / s))
            ps.append(jnp.concatenate(pts, axis=0).T)
        return ps

    def pv(br, g, ps):
        rows = []
        for bb in range(B // 4):
            p = ps[bb]
            lhs = [jnp.concatenate(
                [jnp.where(lane_blk == j, p[h * SQ:(h + 1) * SQ], 0.0) for j in range(4)],
                axis=0).astype(BF) for h in range(G)]
            if br == 0:
                kv = (g * G) // 8
                vs = jnp.concatenate(
                    [av_v[b, kv * SK:(kv + 1) * SK, :] for b in range(4 * bb, 4 * bb + 4)], axis=0)
                os_ = [jnp.dot(lhs[h], vs, preferred_element_type=F32) for h in range(G)]
            else:
                os_ = []
                for h in range(G):
                    vs = jnp.concatenate(
                        [bv_v[g, b, h * SK:(h + 1) * SK, :] for b in range(4 * bb, 4 * bb + 4)], axis=0)
                    os_.append(jnp.dot(lhs[h], vs, preferred_element_type=F32))
            rows.append(jnp.concatenate(os_, axis=1).astype(BF))
        return jnp.concatenate(rows, axis=0)

    out_copies = []

    def oproj(br, g, o):
        r = jnp.dot(o, wo_v[br, g], preferred_element_type=F32)
        if g == 0:
            acc[...] = r
        elif g < NG - 1:
            acc[...] += r
        else:
            o_v[br] = (acc[...] + r).astype(BF)
            c = pltpu.make_async_copy(o_v.at[br], out.at[:, pl.ds(br * D, D)], osems.at[br])
            c.start()
            out_copies.append(c)

    nsteps = len(stages) + 1
    for t in range(min(ahead, nsteps)):
        for n in needs(t):
            copies[n].start()
    ps = None
    for t in range(nsteps):
        for n in needs(t):
            copies[n].wait()
        if t + ahead < nsteps:
            for n in needs(t + ahead):
                copies[n].start()
        if t < len(stages):
            q = qproj(*stages[t])
        if t >= 1:
            o = pv(*stages[t - 1], ps)
        if t < len(stages):
            ps = scores(*stages[t], q)
        if t >= 1:
            oproj(*stages[t - 1], o)
    for c in out_copies:
        c.wait()


def _make(ahead=2):
    @jax.jit
    def f(A_x, A_k_cache, A_v_cache, A_wq, A_wo, B_x, B_k_cache, B_v_cache, B_wq, B_wo):
        hkv = A_k_cache.shape[1]
        anyspec = pl.BlockSpec(memory_space=pl.ANY)
        out = pl.pallas_call(
            functools.partial(_kernel, ahead=ahead),
            out_shape=jax.ShapeDtypeStruct((M, 2 * D), BF),
            in_specs=[anyspec] * 10,
            out_specs=anyspec,
            scratch_shapes=[
                pltpu.VMEM((2, M, D), BF),
                pltpu.VMEM((2, NG, D, G * DH), BF),
                pltpu.VMEM((2, NG, G * DH, D), BF),
                pltpu.VMEM((B, hkv * SK, DH), BF),
                pltpu.VMEM((B, hkv * SK, DH), BF),
                pltpu.VMEM((NG, B, G * SK, DH), BF),
                pltpu.VMEM((NG, B, G * SK, DH), BF),
                pltpu.VMEM((M, D), F32),
                pltpu.VMEM((2, M, D), BF),
                pltpu.SemaphoreType.DMA((64,)),
                pltpu.SemaphoreType.DMA((2,)),
            ],
            compiler_params=pltpu.CompilerParams(vmem_limit_bytes=110 * 2**20),
            name="fused",
        )(A_x.reshape(M, D), A_k_cache.reshape(B, hkv * SK, DH), A_v_cache.reshape(B, hkv * SK, DH),
          A_wq, A_wo,
          B_x.reshape(M, D), B_k_cache.reshape(B, H * SK, DH), B_v_cache.reshape(B, H * SK, DH),
          B_wq, B_wo)
        return out.reshape(B, SQ, 2 * D)
    return f


pallas_concat_heads__gqa_block_cached__mha_block_cached__near_ridge_kernel = _make()
```

```python
import contextlib
import functools
import math
import jax
import jax.numpy as jnp
from jax import lax
import jax.experimental.pallas as pl
import jax.experimental.pallas.tpu as pltpu

B, SQ, D = 16, 32, 1024
H, SK, DH = 32, 32, 128
M = B * SQ
G = 4
NG = H // G
BF = jnp.bfloat16
F32 = jnp.float32
NN = (((1,), (0,)), ((), ()))
NT = (((1,), (1,)), ((), ()))
MB = M // 4

LT = {1: ((0, 1), (3, 1)), 2: ((2, 1), (3, 1)), 3: ((0, 1),), 4: ((3, 1),), 5: ((0, 1), (1, 1)), 6: ((2, 1), (0, -1)), 7: ((1, 1), (3, -1))}
RT = {1: ((0, 1), (3, 1)), 2: ((0, 1),), 3: ((1, 1), (3, -1)), 4: ((2, 1), (0, -1)), 5: ((3, 1),), 6: ((0, 1), (1, 1)), 7: ((2, 1), (3, 1))}
FLIP = {1: 0, 2: 0, 3: 1, 4: 0, 5: 1, 6: 1, 7: 1}

OUT = (lambda m: ((m(4) - m(5)) + m(1)) + m(7), lambda m: m(3) + m(5), lambda m: m(2) + m(4),
       lambda m: ((m(3) - m(2)) + m(1)) + m(6))
NEED = ({1, 4, 5, 7}, {3, 5}, {2, 4}, {1, 2, 3, 6})


def pos(q, e):
    return 2 * (q // 2) + e // 2, 2 * (q % 2) + e % 2


def comb(terms, get):
    v = get(terms[0][0])
    for i, s in terms[1:]:
        v = v + get(i) if s > 0 else v - get(i)
    return v


def operand(ti, tj, outer, base, reassoc):
    once = [e for e, _ in tj if e in (1, 2)]
    if not (reassoc and len(ti) == 2 and once):
        return comb(tj, outer)
    e, = once
    (e2, s2), = [(x, sg) for x, sg in tj if x != e]
    v = base(ti[0][0], e)
    v = v + outer(e2) if s2 > 0 else v - outer(e2)
    return v + base(ti[1][0], e) if ti[1][1] > 0 else v - base(ti[1][0], e)


def ready(order, n):
    return [q for q in range(4) if order[n] in NEED[q] and NEED[q] <= set(order[:n + 1])]


def _kernel(ax, ak, av, awq, awo, bx, bk, bv, bwq, bwo, out,
            x_v, w_v, wo_v, ak_v, av_v, bk_v, bv_v, o_v, out_v, fence_v, sems, osem, *, cfg):
    KH, NH = H * DH // 2, D // 2
    qord, qin, oord, oin = cfg["qord"], cfg["qin"], cfg["oord"], cfg["oin"]
    scope = jax.named_scope if cfg["scope"] else (lambda n: contextlib.nullcontext())
    ns = cfg["split"]
    stages = [(g, (0,)) for g in range(ns)] + [(g, (1,)) for g in range(ns)] + [(g, (0, 1)) for g in range(ns, NG)]

    loads = []
    for g, hfs in stages:
        ks = pl.ds(hfs[0] * NH, len(hfs) * NH)
        if g == 0:
            loads.append(("x", (slice(None), ks)))
        loads.append(("wq", (ks, pl.ds(g * G * DH, G * DH))))
    loads.append(("kv", None))
    wo_quads = []
    for i in oord:
        wo_quads.append([q for q, _ in RT[i] if not any(q in x for x in wo_quads)])
        loads += [("wo", (pl.ds(q // 2 * KH, KH), pl.ds(q % 2 * NH, NH))) for q in wo_quads[-1]]
    bufs = dict(x=x_v, wq=w_v, wo=wo_v)
    kv_bufs = ((ak_v, av_v), (bk_v, bv_v))
    for br, srcs in enumerate((dict(x=ax, wq=awq, wo=awo, kv=(ak, av)), dict(x=bx, wq=bwq, wo=bwo, kv=(bk, bv)))):
        for n, (kind, sl) in enumerate(loads):
            if kind == "kv":
                for src, dst in zip(srcs[kind], kv_bufs[br]):
                    pltpu.make_async_copy(src, dst, sems.at[br, n]).start()
            else:
                pltpu.make_async_copy(srcs[kind].at[sl], bufs[kind].at[br].at[sl], sems.at[br, n]).start()

    def fence():
        fence_v[...] = jnp.zeros((8, 128), F32)

    lane_blk = lax.broadcasted_iota(jnp.int32, (SK, 128), 1) // 32
    scale = DH ** -0.5 * math.log2(math.e)

    def attention(br, n):
        k_v, v_v = kv_bufs[br]
        with scope(f"wkv{br}"):
            for dst in kv_bufs[br]:
                pltpu.make_async_copy(dst, dst, sems.at[br, n]).wait()

        @functools.cache
        def probs(g, b):
            qq = jnp.concatenate([o_v[b * SQ:(b + 1) * SQ, h * DH:(h + 1) * DH] for h in range(g * G, (g + 1) * G)], axis=0).astype(BF)
            if br == 0:
                kv = (g * G) // 8
                st = lax.dot_general(k_v[b, kv * SK:(kv + 1) * SK, :], qq, NT, preferred_element_type=F32)
            else:
                full = lax.dot_general(k_v[b, g * G * SK:(g + 1) * G * SK, :], qq, NT, preferred_element_type=F32)
                st = full[0:SK]
                for j in range(1, G):
                    st = jnp.where(lane_blk == j, full[j * SK:(j + 1) * SK], st)
            m = jnp.max(st, axis=0, keepdims=True)
            e = jnp.exp2((st - m) * scale)
            return e * (1.0 / jnp.sum(e, axis=0, keepdims=True))

        def pv(g, bb):
            p = jnp.concatenate([probs(g, 4 * bb + i) for i in range(4)], axis=0).T
            for h in range(G):
                hh = g * G + h
                lhs = jnp.concatenate(
                    [jnp.where(lane_blk == j, p[h * SQ:(h + 1) * SQ], 0.0) for j in range(4)], axis=0)
                if cfg["ppack"]:
                    lhs = lhs.astype(BF)
                kv = hh if br else hh // 8
                vs = v_v[4 * bb:4 * bb + 4, kv * SK:(kv + 1) * SK, :]
                o_v[bb * MB:(bb + 1) * MB, hh * DH:(hh + 1) * DH] = lax.dot_general(
                    lhs, vs.reshape(4 * SK, DH), NN, preferred_element_type=F32)

        tiles = [(g, bb) for g in range(NG) for bb in range(4)]
        lag = cfg["lag"][br]
        for t in range(len(tiles) + lag):
            if t < len(tiles):
                for i in range(4):
                    probs(tiles[t][0], 4 * tiles[t][1] + i)
            if t >= lag:
                pv(*tiles[t - lag])

    @pl.loop(0, 2)
    def _(br):
        pending = list(enumerate(loads))

        def wait(kind):
            n, (k, sl) = pending.pop(0)
            assert k == kind
            dst = bufs[kind].at[br].at[sl]
            pltpu.make_async_copy(dst, dst, sems.at[br, n]).wait()

        @functools.cache
        def x_blk(r, c, hf, use):
            return x_v[br, r * MB:(r + 1) * MB, hf * NH + c * 128:hf * NH + (c + 1) * 128].astype(F32)

        def x_base(i, q, e, hf):
            return x_blk(*pos(q, e), hf, i if q in cfg["xremat"] else 0)

        @functools.cache
        def x_outer(i, e, hf):
            return comb(LT[i], lambda q: x_base(i, q, e, hf))

        @functools.cache
        def x_op(i, j, hf):
            return operand(LT[i], LT[j], lambda e: x_outer(i, e, hf), lambda q, e: x_base(i, q, e, hf), i in cfg["xre"]).astype(BF)

        @functools.cache
        def wq_blk(g, r, c, hf, use):
            return w_v[br, hf * NH + r * 128:hf * NH + (r + 1) * 128, (g * G + c) * DH:(g * G + c + 1) * DH].astype(F32)

        def wq_base(g, i, q, e, hf):
            return wq_blk(g, *pos(q, e), hf, i if q in cfg["remat"] else 0)

        @functools.cache
        def wq_outer(g, i, e, hf):
            return comb(RT[i], lambda q: wq_base(g, i, q, e, hf))

        @functools.cache
        def qprod(g, i, j, hf):
            acc = qprod(g, i, j, 0) if hf and not (g < ns and cfg["cacc"]) else None
            rhs = operand(RT[i], RT[j], lambda e: wq_outer(g, i, e, hf), lambda q, e: wq_base(g, i, q, e, hf), i in cfg["qre"])
            d = lax.dot_general(x_op(i, j, hf), rhs, NN, preferred_element_type=F32)
            return d if acc is None else d + acc

        @functools.cache
        def qmid(g, i, e, hf):
            return OUT[e](lambda j: qprod(g, i, j, hf))

        for g, hfs in stages:
            if g == 0:
                wait("x")
            wait("wq")
            for a, i in enumerate(qord):
                fence()
                for n, j in enumerate(qin):
                    qprod(g, i, j, hfs[-1])
                    if hfs[-1] or cfg["cacc"]:
                        for e in ready(qin, n):
                            for q in ready(qord, a):
                                r, c = pos(q, e)
                                v = OUT[q](lambda u: qmid(g, u, e, hfs[-1]))
                                sl = (slice(r * MB, (r + 1) * MB), slice((g * G + c) * DH, (g * G + c + 1) * DH))
                                o_v[sl] = o_v[sl] + v if hfs == (1,) and cfg["cacc"] else v

        n, _ = pending.pop(0)
        lax.cond(br == 0, lambda: attention(0, n), lambda: attention(1, n))

        KO, NO, KC = H * DH // 4, D // 4, cfg["kc"]

        def o_blk(r, c, t):
            return o_v[r * MB:(r + 1) * MB, c * KO + t * KC:c * KO + (t + 1) * KC]

        @functools.cache
        def wo_blk(q, e, t, use):
            r, c = pos(q, e)
            return wo_v[br, r * KO + t * KC:r * KO + (t + 1) * KC, c * NO:(c + 1) * NO].astype(F32)

        def wo_base(i, q, e, t):
            return wo_blk(q, e ^ FLIP[i], t, i if q in cfg["oremat"] else 0)

        @functools.cache
        def o_outer(i, e, t, use):
            return comb(LT[i], lambda q: o_blk(*pos(q, e), t))

        @functools.cache
        def wo_outer(i, e, t):
            return comb(RT[i], lambda q: wo_base(i, q, e, t))

        @functools.cache
        def oprod(i, j):
            acc = None
            for t in range(KO // KC):
                lhs = operand(LT[i], LT[j], lambda e: o_outer(i, e, t, j if len(LT[i]) == 1 else 0),
                              lambda q, e: o_blk(*pos(q, e), t), True)
                rhs = operand(RT[i], RT[j], lambda e: wo_outer(i, e, t), lambda q, e: wo_base(i, q, e, t), i in cfg["ore"])
                d = lax.dot_general(lhs, rhs, NN, preferred_element_type=F32)
                acc = d if acc is None else d + acc
            return acc

        @functools.cache
        def omid(i, e):
            return OUT[e ^ FLIP[i]](lambda j: oprod(i, j))

        def flush(r0, nr, c0, nc):
            pltpu.make_async_copy(out_v.at[br, pl.ds(r0, nr), pl.ds(c0, nc)],
                                  out.at[pl.ds(r0, nr), pl.ds(pl.multiple_of(br * D + c0, NO), nc)], osem).start()

        for a, i in enumerate(oord):
            for _ in wo_quads[a]:
                wait("wo")
            for n, j in enumerate(oin):
                fence()
                oprod(i, j)
                for e in ready(oin, n):
                    for q in ready(oord, a):
                        r, c = pos(q, e ^ FLIP[i])
                        out_v[br, r * MB:(r + 1) * MB, c * NO:(c + 1) * NO] = OUT[q](lambda u: omid(u, e ^ FLIP[i])).astype(BF)
                        if a == 6:
                            flush(r * MB, MB, c * NO, NO)
            for q in ready(oord, a):
                if a < 6:
                    flush(q // 2 * 2 * MB, 2 * MB, q % 2 * NH, NH)
        assert not pending

    with scope("wend"):
        pltpu.make_async_copy(out_v, out_v, osem).wait()


def _make(flags={'XLA_TPU_RESCHEDULE_DMA_DONES': True}, cp={}, **kw):
    o = (2, 4, 5, 3, 1, 7, 6)
    cfg = dict(qre=(1,), ore=(), kc=256, remat=(1, 2), oremat=(1, 2), split=0, scope=0, ppack=0, cacc=0,
               xre=(), xremat=(0, 1, 2, 3), qord=o, qin=o, oord=o, oin=o, lag=(4, 3))
    assert set(kw) <= set(cfg)
    cfg.update(kw)

    @jax.jit
    def f(A_x, A_k_cache, A_v_cache, A_wq, A_wo, B_x, B_k_cache, B_v_cache, B_wq, B_wo):
        hkv = A_k_cache.shape[1]
        anyspec = pl.BlockSpec(memory_space=pl.ANY)
        out = pl.pallas_call(
            functools.partial(_kernel, cfg=cfg),
            out_shape=jax.ShapeDtypeStruct((M, 2 * D), BF),
            in_specs=[anyspec] * 10,
            out_specs=anyspec,
            scratch_shapes=[
                pltpu.VMEM((2, M, D), BF),
                pltpu.VMEM((2, D, H * DH), BF),
                pltpu.VMEM((2, H * DH, D), BF),
                pltpu.VMEM((B, hkv * SK, DH), BF),
                pltpu.VMEM((B, hkv * SK, DH), BF),
                pltpu.VMEM((B, H * SK, DH), BF),
                pltpu.VMEM((B, H * SK, DH), BF),
                pltpu.VMEM((M, H * DH), F32),
                pltpu.VMEM((2, M, D), BF),
                pltpu.VMEM((8, 128), F32),
                pltpu.SemaphoreType.DMA((2, 14 + cfg["split"] + bool(cfg["split"]))),
                pltpu.SemaphoreType.DMA(()),
            ],
            compiler_params=pltpu.CompilerParams(vmem_limit_bytes=120 * 2**20, flags=flags, **cp),
            name="fused",
        )(A_x.reshape(M, D), A_k_cache.reshape(B, hkv * SK, DH), A_v_cache.reshape(B, hkv * SK, DH),
          A_wq, A_wo,
          B_x.reshape(M, D), B_k_cache.reshape(B, H * SK, DH), B_v_cache.reshape(B, H * SK, DH),
          B_wq, B_wo)
        return out.reshape(B, SQ, 2 * D)
    return f


pallas_concat_heads__gqa_block_cached__mha_block_cached__near_ridge_kernel = _make(lag=(6,4), ppack=1, split=3)
```

```python
import functools
import itertools
import math

import jax
import jax.numpy as jnp
from jax import lax
import jax.experimental.pallas as pl
import jax.experimental.pallas.tpu as pltpu

B, SQ, D = 16, 32, 1024
H, HKV, SK, DH = 32, 4, 32, 128
REP = H // HKV
M = B * SQ

PASSES = 2
HP = H // PASSES
G = 4
STAGES = HP // G
KVP = HKV // PASSES
W = G * DH
COLS = D // DH

K_CUTS = (0, 128, 256, 384, 512, D)
CUT_STAGES = 3
MXU_BATCHES = (12, 0)
PV_LAG = 4
MHA_SCORES_AT = 23
EARLY_COLS = 5
VPU_KEYS = 6
VPU_FROM, VPU_SLACK = 43, 2
TAIL_COLS = (0, 4, 6, 7, 8)
TAIL_ROWS = (0, 256, 384, 448, M)

BF16 = jnp.bfloat16
F32 = jnp.float32
NT = (((1,), (1,)), ((), ()))
CHUNKS = tuple(zip(K_CUTS, K_CUTS[1:]))
SLICES = -(-SK // VPU_KEYS)
NUM_LOADS = len(CHUNKS) * (1 + CUT_STAGES) + (STAGES - CUT_STAGES) + 1 + STAGES + 4 + 2 * STAGES


def _aligned(start, size, align):
    return pl.ds(pl.multiple_of(start, align), size)


def _kernel(ax, ak, av, awq, awo, bx, bk, bv, bwq, bwo, out,
            x_v, w_v, ak_v, av_v, bk_v, bv_v, acc_v, out_v, vf_v, load_sems, store_sem):

    def loads(t):
        r = []

        def add(use, src, dst):
            r.append((use, pltpu.make_async_copy(src, dst, load_sems.at[t, len(r)])))

        def add_wq(wq, br, s, k0, k1):
            ks = pl.ds(k0, k1 - k0)
            add(("q", br, k0, s * G), wq.at[ks, _aligned((t * STAGES + s) * W, W, W)], w_v.at[t, br, s, ks])

        def add_cache(src, dst):
            n = src.shape[1] // PASSES
            add(r[-1][0], src.at[:, _aligned(t * n, n, n)], dst.at[t])

        for k0, k1 in CHUNKS:
            ks = pl.ds(k0, k1 - k0)
            add(("q", 0, k0, 0), ax.at[:, ks], x_v.at[t, 0, :, ks])
            for s in range(CUT_STAGES):
                add_wq(awq, 0, s, k0, k1)
                if (k1, s) == (D, 1):
                    add_cache(ak, ak_v)
                    add_cache(av, av_v)
        for s in range(CUT_STAGES, STAGES):
            add_wq(awq, 0, s, 0, D)
        add(("q", 1, 0, 0), bx, x_v.at[t, 1])
        for s in range(STAGES):
            add_wq(bwq, 1, s, 0, D)
            if s == STAGES - 2:
                add_cache(bk, bk_v)
            if s == STAGES - 1:
                add_cache(bv, bv_v)
        for br, wo in ((1, bwo), (0, awo)):
            for s in range(0, STAGES, 2):
                for c in range(2):
                    add(("o", br, s, c * G), wo.at[_aligned((t * STAGES + s) * W, 2 * W, W), pl.ds(c * W, W)],
                        w_v.at[t, 2 + br, s + c])
        assert len(r) == NUM_LOADS
        return r

    @pl.loop(0, PASSES)
    def _(t):
        for _, copy in loads(t):
            copy.start()

    lane_group = lax.broadcasted_iota(jnp.int32, (SK, G * SQ), 1) // SQ
    scale = DH ** -0.5 * math.log2(math.e)

    @pl.loop(0, PASSES)
    def _(t):
        pending = loads(t)
        q, probs, o, partial = {}, {}, {}, {}
        latest = [None]
        slot = jnp.minimum(t, PASSES - 1)

        def wait(use):
            while any(u == use for u, _ in pending):
                pending.pop(0)[1].wait()

        def q_proj(br, h, nh, k0, k1):
            wait(("q", br, k0, h))
            c = h % G * DH
            r = jnp.dot(x_v[t, br, :, k0:k1], w_v[t, br, h // G, k0:k1, c:c + nh * DH],
                        preferred_element_type=F32)
            if k0:
                r = r + jnp.concatenate([q[br, h + j] for j in range(nh)], axis=1)
            latest[0] = r
            for j in range(nh):
                q[br, h + j] = r[:, j * DH:(j + 1) * DH]

        def softmax(br, s, bb):
            exps = []
            for b in range(bb * G, (bb + 1) * G):
                qs = jnp.concatenate([q[br, s * G + j][b * SQ:(b + 1) * SQ] for j in range(G)],
                                     axis=0).astype(BF16)
                if br == 0:
                    kv = s * G // REP
                    st = lax.dot_general(ak_v[t, b, kv * SK:(kv + 1) * SK, :], qs, NT,
                                         preferred_element_type=F32)
                else:
                    full = lax.dot_general(bk_v[t, b, s * G * SK:(s + 1) * G * SK, :], qs, NT,
                                           preferred_element_type=F32)
                    st = full[:SK]
                    for j in range(1, G):
                        st = jnp.where(lane_group == j, full[j * SK:(j + 1) * SK], st)
                exps.append(jnp.exp2((st - jnp.max(st, axis=0, keepdims=True)) * scale))
            inv = 1.0 / jnp.concatenate([jnp.sum(e, axis=0, keepdims=True) for e in exps], axis=0)
            for i, e in enumerate(exps):
                probs[br, s, bb * G + i] = e * inv[i:i + 1]

        def pv_mxu(br, s, bb):
            p = jnp.concatenate([probs[br, s, b] for b in range(bb * G, (bb + 1) * G)], axis=0).T
            for j in range(G):
                h = s * G + j
                lhs = jnp.concatenate([jnp.where(lane_group == i, p[j * SQ:(j + 1) * SQ], 0.0)
                                       for i in range(G)], axis=0).astype(BF16)
                v_v, kv = (bv_v, h) if br else (av_v, h // REP)
                v = v_v[t, bb * G:(bb + 1) * G, kv * SK:(kv + 1) * SK, :].reshape(G * SK, DH)
                r = jnp.dot(lhs, v, preferred_element_type=F32)
                for i in range(G):
                    o[br, h, bb * G + i] = r[i * SQ:(i + 1) * SQ]

        def pv_vpu(kv, b):
            vf_v[t, kv, b, :SK] = av_v[t, b, kv * SK:(kv + 1) * SK, :].astype(F32)
            stages = range(kv * REP // G, (kv + 1) * REP // G)
            acc = {}
            for k in range(SK):
                if k % VPU_KEYS == 0:
                    if k:
                        yield
                    row = SK + k // VPU_KEYS * 8
                    vf_v[t, kv, b, row:row + 8] = latest[0][-8:, :DH]
                col = jnp.broadcast_to(vf_v[slot, kv, b, k:k + 1, :], (G * SQ, DH)).T
                for s in stages:
                    term = col * probs[0, s, b][k:k + 1]
                    acc[s] = acc[s] + term if k else term
            for s in stages:
                r = acc[s].T
                for j in range(G):
                    o[0, s * G + j, b] = r[j * SQ:(j + 1) * SQ]
            yield

        @functools.cache
        def o_stage(br, s):
            rows = [jnp.concatenate([o[br, h, b] for h in range(s * G, (s + 1) * G)], axis=1)
                    for b in range(B)]
            return jnp.concatenate(rows, axis=0).astype(BF16)

        def store(br, r0, r1, c0, c1):
            @pl.when(t == PASSES - 1)
            def _():
                rows, n = pl.ds(r0, r1 - r0), (c1 - c0) * DH
                pltpu.make_async_copy(out_v.at[br, rows, pl.ds(c0 * DH, n)],
                                      out.at[rows, pl.ds(br * D + c0 * DH, n)], store_sem).start()

        def o_proj(br, c, s):
            wait(("o", br, s, c))
            cols = slice(c * DH, (c + 1) * DH)
            prev = partial[br, c] if s else jnp.where(t > 0, acc_v[br, :, cols], 0.0)
            wo = w_v[t, 2 + br, s // 2 * 2 + c // G, s % 2 * W:(s % 2 + 1) * W, c % G * DH:(c % G + 1) * DH]
            r = jnp.dot(o_stage(br, s), wo, preferred_element_type=F32) + prev
            partial[br, c] = latest[0] = r
            if s == STAGES - 1:
                acc_v[br, :, cols] = r
                cuts = TAIL_ROWS if (br, c) == (0, COLS - 1) else (0, M)
                for r0, r1 in zip(cuts, cuts[1:]):
                    out_v[br, r0:r1, cols] = r[r0:r1].astype(BF16)
                    if br == 0 and c + 1 in TAIL_COLS:
                        store(br, r0, r1, max(x for x in TAIL_COLS if x <= c), c + 1)

        for k0, k1 in CHUNKS[:-1]:
            for s in range(CUT_STAGES):
                q_proj(0, s * G, G, k0, k1)

        half = D // 2
        steps = [(q_proj, 0, h, 1, k, k + half)
                 for h in range(HP) for k in (0, half) if k or h >= CUT_STAGES * G]
        b_start = len(steps)
        steps += [(q_proj, 1, h, 1, k, k + half) for h in range(HP) for k in (0, half)]
        steps += [(o_proj, 1, c, s) for s in range(STAGES) for c in range(EARLY_COLS)]
        steps += [(o_proj, 1, c, s) for c in range(EARLY_COLS, COLS) for s in range(STAGES)]
        steps += [(o_proj, 0, c, s) for s0 in range(0, STAGES, 2) for c in range(COLS) for s in (s0, s0 + 1)]

        between = [[] for _ in steps]
        for kv, first in enumerate((REP, b_start)):
            tiles = [(s, bb) for bb in range(B // G) for s in range(kv * REP // G, (kv + 1) * REP // G)]
            for i, (s, bb) in enumerate(tiles, first):
                between[i].append((softmax, 0, s, bb))
                if bb * G < MXU_BATCHES[kv]:
                    between[i + PV_LAG].insert(0, (pv_mxu, 0, s, bb))
        tiles = [(s, bb) for s in range(STAGES) for bb in range(B // G)]
        for i, (s, bb) in enumerate(tiles, b_start + MHA_SCORES_AT):
            between[i].append((softmax, 1, s, bb))
            between[i + PV_LAG].insert(0, (pv_mxu, 1, s, bb))
        between[-12].append((store, 1, 0, M, 0, COLS))

        pairs = [(kv, b) for kv in range(KVP) for b in range(MXU_BATCHES[kv], B)]
        vpu_work = itertools.chain(*[pv_vpu(kv, b) for kv, b in pairs])
        total, done = len(pairs) * SLICES, 0
        span = len(steps) - 2 * COLS - VPU_SLACK - VPU_FROM
        for i, step in enumerate(steps):
            for fn, *args in [step] + between[i]:
                fn(*args)
            while done < total and done * span <= (i - VPU_FROM) * total:
                next(vpu_work)
                done += 1
        assert not pending

    pltpu.make_async_copy(out, out, store_sem).wait()


@jax.jit
def pallas_concat_heads__gqa_block_cached__mha_block_cached__near_ridge_kernel(
    A_x: jax.Array,
    A_k_cache: jax.Array,
    A_v_cache: jax.Array,
    A_wq: jax.Array,
    A_wo: jax.Array,
    B_x: jax.Array,
    B_k_cache: jax.Array,
    B_v_cache: jax.Array,
    B_wq: jax.Array,
    B_wo: jax.Array,
):
    in_hbm = pl.BlockSpec(memory_space=pl.ANY)
    out = pl.pallas_call(
        _kernel,
        out_shape=jax.ShapeDtypeStruct((M, 2 * D), BF16),
        in_specs=[in_hbm] * 10,
        out_specs=in_hbm,
        scratch_shapes=[
            pltpu.VMEM((PASSES, 2, M, D), BF16),
            pltpu.VMEM((PASSES, 4, STAGES, D, W), BF16),
            pltpu.VMEM((PASSES, B, KVP * SK, DH), BF16),
            pltpu.VMEM((PASSES, B, KVP * SK, DH), BF16),
            pltpu.VMEM((PASSES, B, HP * SK, DH), BF16),
            pltpu.VMEM((PASSES, B, HP * SK, DH), BF16),
            pltpu.VMEM((2, M, D), F32),
            pltpu.VMEM((2, M, D), BF16),
            pltpu.VMEM((PASSES, KVP, B, SK + 8 * SLICES, DH), F32),
            pltpu.SemaphoreType.DMA((PASSES, NUM_LOADS)),
            pltpu.SemaphoreType.DMA(()),
        ],
        compiler_params=pltpu.CompilerParams(
            vmem_limit_bytes=100 * 2**20,
            disable_semaphore_checks=True,
            flags={"XLA_TPU_RESCHEDULE_DMA_DONES": True},
        ),
        name="fused",
    )(
        A_x.reshape(M, D), A_k_cache.reshape(B, HKV * SK, DH), A_v_cache.reshape(B, HKV * SK, DH), A_wq, A_wo,
        B_x.reshape(M, D), B_k_cache.reshape(B, H * SK, DH), B_v_cache.reshape(B, H * SK, DH), B_wq, B_wo,
    )
    return out.reshape(B, SQ, 2 * D)
```
